```python
import os as _os
_os.environ.setdefault("JAX_PLATFORMS", "cpu")
import jax
import jax.numpy as jnp

def _softmax(x, axis=-1):
    return jax.nn.softmax(x, axis=axis)
def _gelu(x):
    return jax.nn.gelu(x, approximate=True)
def _silu(x):
    return jax.nn.silu(x)
def _sigmoid(x):
    return jax.nn.sigmoid(x)
def _layernorm(x, axis=-1, eps=1e-5):
    m = jnp.mean(x, axis=axis, keepdims=True)
    v = jnp.var(x, axis=axis, keepdims=True)
    return (x - m) / jnp.sqrt(v + eps)
def _scatter_add(tgt, idx, src, axis=0):
    return tgt.at[idx].add(src)
def _segment_sum(src, seg, n):
    return jax.ops.segment_sum(src, seg, n)
class _Rng:
    def __init__(self, key):
        self._k = key
    def _next(self):
        self._k, sub = jax.random.split(self._k)
        return sub
    def normal(self, shape):
        return jax.random.normal(self._next(), shape, dtype=jnp.bfloat16)
    def randint(self, lo, hi, shape):
        return jax.random.randint(self._next(), shape, lo, hi, dtype=jnp.int32)
    def uniform(self, shape, lo=0.0, hi=1.0):
        return jax.random.uniform(self._next(), shape, jnp.bfloat16, lo, hi)
    def permutation(self, n):
        return jax.random.permutation(self._next(), n)


kernel_name = 'standalone__dense_activation_gelu__prompt'

def setup_inputs():
    _rng = _Rng(jax.random.key(int.from_bytes(__import__("os").urandom(4), "little")))
    _w = (lambda a: (lambda t: t.astype(jnp.bfloat16) if jnp.issubdtype(t.dtype, jnp.floating) else t)(jnp.asarray(a)))
    B, S, D, F = 1, 2048, 640, 1728
    return {
        "x": _w((lambda *s: _rng.normal(s) * 0.05)(B, S, D)),
        "w1": _w((lambda *s: _rng.normal(s) * 0.05)(D, F) * (D ** -0.5)),
        "b1": _w((lambda *s: _rng.normal(s) * 0.05)(F) * 0.01),
        "w2": _w((lambda *s: _rng.normal(s) * 0.05)(F, D) * (F ** -0.5)),
        "b2": _w((lambda *s: _rng.normal(s) * 0.05)(D) * 0.01),
    }

def reference(x, w1, b1, w2, b2):
    h = jnp.einsum("bsd,df->bsf", x, w1) + b1
    h = _gelu(h)
    return jnp.einsum("bsf,fd->bsd", h, w2) + b2
```

```python
import functools

import jax
import jax.numpy as jnp
import jax.experimental.pallas as pl
import jax.experimental.pallas.tpu as pltpu


def _mlp_kernel(x_ref, w1_ref, b1_ref, w2_ref, b2_ref, o_ref):
    h = jnp.dot(x_ref[...], w1_ref[...], preferred_element_type=jnp.float32)
    h = h + b1_ref[...].astype(jnp.float32)
    h = jax.nn.gelu(h, approximate=True)
    y = jnp.dot(h.astype(jnp.bfloat16), w2_ref[...],
                preferred_element_type=jnp.float32)
    y = y + b2_ref[...].astype(jnp.float32)
    o_ref[...] = y.astype(o_ref.dtype)


TM = 256


@jax.jit
def pallas_standalone__dense_activation_gelu__prompt_kernel(
    x: jax.Array,
    w1: jax.Array,
    b1: jax.Array,
    w2: jax.Array,
    b2: jax.Array,
):
    B, S, D = x.shape
    F = w1.shape[1]
    M = B * S
    x2 = x.reshape(M, D)
    b1_2 = b1.reshape(1, F)
    b2_2 = b2.reshape(1, D)
    tm = min(TM, M)
    assert M % tm == 0

    out = pl.pallas_call(
        _mlp_kernel,
        grid=(M // tm,),
        in_specs=[
            pl.BlockSpec((tm, D), lambda i: (i, 0)),
            pl.BlockSpec((D, F), lambda i: (0, 0)),
            pl.BlockSpec((1, F), lambda i: (0, 0)),
            pl.BlockSpec((F, D), lambda i: (0, 0)),
            pl.BlockSpec((1, D), lambda i: (0, 0)),
        ],
        out_specs=pl.BlockSpec((tm, D), lambda i: (i, 0)),
        out_shape=jax.ShapeDtypeStruct((M, D), x.dtype),
        compiler_params=pltpu.CompilerParams(
            dimension_semantics=("parallel",),
            vmem_limit_bytes=100 * 1024 * 1024,
        ),
    )(x2, w1, b1_2, w2, b2_2)
    return out.reshape(B, S, D)
```

```python
import numpy as np

import jax
import jax.numpy as jnp
import jax.experimental.pallas as pl
import jax.experimental.pallas.tpu as pltpu

_NT_DIMS = (((1,), (1,)), ((), ()))

_TM = 256
_CHUNKS_BY_F = {1728: (64, 192, 448, 512, 512)}


def _make_kernel(offsets, chunks):
    n_chunks = len(chunks)

    def kernel(x_ref, w1t_hbm, b1_ref, w2_hbm, b2_ref, o_ref,
               w1t_vmem, w2_vmem, sems):
        step = pl.program_id(0)

        def weight_copy(c, which):
            src, dst = (w1t_hbm, w1t_vmem) if which == 0 else (w2_hbm, w2_vmem)
            rows = pl.ds(offsets[c], chunks[c])
            return pltpu.make_async_copy(src.at[rows], dst.at[rows],
                                         sems.at[which, c])

        b2 = b2_ref[...].astype(jnp.float32).reshape(1, -1)

        @pl.when(step == 0)
        def _first_step():
            for c in range(n_chunks):
                weight_copy(c, 0).start()
                weight_copy(c, 1).start()
            x = x_ref[...]
            b1 = b1_ref[...].astype(jnp.float32).reshape(1, -1)
            acc = None
            for c in range(n_chunks):
                weight_copy(c, 0).wait()
                weight_copy(c, 1).wait()
                lo, n = offsets[c], chunks[c]
                h = jax.lax.dot_general(x, w1t_vmem[lo:lo + n, :], _NT_DIMS,
                                        preferred_element_type=jnp.float32)
                h = jax.nn.gelu(h + b1[:, lo:lo + n], approximate=True)
                part = jnp.dot(h.astype(jnp.bfloat16), w2_vmem[lo:lo + n, :],
                               preferred_element_type=jnp.float32)
                acc = part if acc is None else acc + part
            o_ref[...] = (acc + b2).astype(o_ref.dtype)

        @pl.when(step > 0)
        def _steady_state():
            h = jax.lax.dot_general(x_ref[...], w1t_vmem[...], _NT_DIMS,
                                    preferred_element_type=jnp.float32)
            h = h + b1_ref[...].astype(jnp.float32).reshape(1, -1)
            h = jax.nn.gelu(h, approximate=True)
            y = jnp.dot(h.astype(jnp.bfloat16), w2_vmem[...],
                        preferred_element_type=jnp.float32)
            o_ref[...] = (y + b2).astype(o_ref.dtype)

    return kernel


@jax.jit
def pallas_standalone__dense_activation_gelu__prompt_kernel(
    x: jax.Array,
    w1: jax.Array,
    b1: jax.Array,
    w2: jax.Array,
    b2: jax.Array,
):
    B, S, D = x.shape
    F = w1.shape[1]
    M = B * S

    tm = _TM if M % _TM == 0 else M
    chunks = _CHUNKS_BY_F.get(F, (F,))
    assert sum(chunks) == F, "weight chunks must cover all of F"
    offsets = tuple(int(o) for o in np.cumsum((0,) + tuple(chunks))[:-1])
    n_chunks = len(chunks)

    out = pl.pallas_call(
        _make_kernel(offsets, chunks),
        grid=(M // tm,),
        in_specs=[
            pl.BlockSpec((tm, D), lambda i: (i, 0)),
            pl.BlockSpec(memory_space=pl.ANY),
            pl.BlockSpec((F,), lambda i: (0,)),
            pl.BlockSpec(memory_space=pl.ANY),
            pl.BlockSpec((D,), lambda i: (0,)),
        ],
        out_specs=pl.BlockSpec((tm, D), lambda i: (i, 0)),
        out_shape=jax.ShapeDtypeStruct((M, D), x.dtype),
        scratch_shapes=[
            pltpu.VMEM((F, D), jnp.bfloat16),
            pltpu.VMEM((F, D), jnp.bfloat16),
            pltpu.SemaphoreType.DMA((2, n_chunks)),
        ],
        compiler_params=pltpu.CompilerParams(
            dimension_semantics=("arbitrary",),
            vmem_limit_bytes=100 * 1024 * 1024,
        ),
    )(x.reshape(M, D), w1.T, b1, w2, b2)
    return out.reshape(B, S, D)
```
